```python
import os as _os
_os.environ.setdefault("JAX_PLATFORMS", "cpu")
import jax
import jax.numpy as jnp

def _softmax(x, axis=-1):
    return jax.nn.softmax(x, axis=axis)
def _gelu(x):
    return jax.nn.gelu(x, approximate=True)
def _silu(x):
    return jax.nn.silu(x)
def _sigmoid(x):
    return jax.nn.sigmoid(x)
def _layernorm(x, axis=-1, eps=1e-5):
    m = jnp.mean(x, axis=axis, keepdims=True)
    v = jnp.var(x, axis=axis, keepdims=True)
    return (x - m) / jnp.sqrt(v + eps)
def _scatter_add(tgt, idx, src, axis=0):
    return tgt.at[idx].add(src)
def _segment_sum(src, seg, n):
    return jax.ops.segment_sum(src, seg, n)
class _Rng:
    def __init__(self, key):
        self._k = key
    def _next(self):
        self._k, sub = jax.random.split(self._k)
        return sub
    def normal(self, shape):
        return jax.random.normal(self._next(), shape, dtype=jnp.bfloat16)
    def randint(self, lo, hi, shape):
        return jax.random.randint(self._next(), shape, lo, hi, dtype=jnp.int32)
    def uniform(self, shape, lo=0.0, hi=1.0):
        return jax.random.uniform(self._next(), shape, jnp.bfloat16, lo, hi)
    def permutation(self, n):
        return jax.random.permutation(self._next(), n)


kernel_name = 'parallel_sum__spectral_gfnet__glu_gated_swiglu__prompt'

def setup_inputs():
    _rng = _Rng(jax.random.key(int.from_bytes(__import__("os").urandom(4), "little")))
    _w = (lambda a: (lambda t: t.astype(jnp.bfloat16) if jnp.issubdtype(t.dtype, jnp.floating) else t)(jnp.asarray(a)))
    def _A_setup():
        B, S, D = 1, 2048, 512
        Df = D // 2 + 1
        return {
            "x": _w((lambda *s: _rng.normal(s) * 0.05)(B, S, D)),
            "w_r": _w((lambda *s: _rng.normal(s) * 0.2)(S, Df) * 0.02),
            "w_i": _w((lambda *s: _rng.normal(s) * 0.2)(S, Df) * 0.02),
        }
    _A_in = _A_setup()

    def _B_setup():
        B, S, D, F = 1, 2048, 512, 1376
        return {
            "x": _w((lambda *s: _rng.normal(s) * 0.05)(B, S, D)),
            "w1": _w((lambda *s: _rng.normal(s) * 0.05)(D, F) * (2.0 / D) ** 0.5),
            "w3": _w((lambda *s: _rng.normal(s) * 0.05)(D, F) * (2.0 / D) ** 0.5),
            "w2": _w((lambda *s: _rng.normal(s) * 0.05)(F, D) * (2.0 / F) ** 0.5),
        }
    _B_in = _B_setup()

    return {
        "A_x": _A_in["x"],
        "A_w_r": _A_in["w_r"],
        "A_w_i": _A_in["w_i"],
        "B_x": _B_in["x"],
        "B_w1": _B_in["w1"],
        "B_w3": _B_in["w3"],
        "B_w2": _B_in["w2"],
    }

def reference(A_x, A_w_r, A_w_i, B_x, B_w1, B_w3, B_w2):
    def _A_ref(x, w_r, w_i):
        B, S, D = x.shape
        X = (lambda x, axes=(-2,-1): jnp.fft.rfft2(x.astype(jnp.float32), axes=axes))(x, axes=(-2, -1))
        W = w_r + 1j * w_i
        X = X * W
        y = (lambda x, s, axes=(-2,-1): jnp.fft.irfft2(x, s=s, axes=axes).astype(jnp.bfloat16))(X, (S, D), axes=(-2, -1))
        return y

    def _B_ref(x, w1, w3, w2):
        gate = jnp.einsum("bsd,df->bsf", x, w1)
        up = jnp.einsum("bsd,df->bsf", x, w3)
        h = _silu(gate) * up
        out = jnp.einsum("bsf,fd->bsd", h, w2)
        return out

    x = A_x
    xn = _layernorm(x, axis=-1)
    return x + _A_ref(xn, A_w_r, A_w_i) + _B_ref(xn, B_w1, B_w3, B_w2)
```

```python
import numpy as np
import jax
import jax.numpy as jnp
import jax.experimental.pallas as pl
import jax.experimental.pallas.tpu as pltpu

S, D, F = 2048, 512, 1376
TM = 256
R = 264
f32, bf16 = jnp.float32, jnp.bfloat16


def _consts():
    n = np.arange(128)
    j = np.arange(64)
    E = lambda l: np.exp(-2j * np.pi * np.outer(l, n) / D)
    e0, e2, e1, e3 = E(4 * j), E(4 * j + 2), E(4 * j + 1), E(4 * j + 3)
    a0 = np.concatenate([e0.real, e0.imag])
    a0[64] = (-1.0) ** n
    a2 = np.concatenate([e2.real, e2.imag])
    a13 = np.block([[e1.real, e1.imag], [e3.real, -e3.imag],
                    [e1.imag, -e1.real], [e3.imag, e3.real]])
    fd = np.block([[a0, a2], [a13]])
    s0 = np.full((128, 1), 2.0)
    s0[0] = s0[64] = 1.0
    gd = np.block([[a0 * s0, 2 * a2], [2 * a13]]) / D
    ms = []
    for a in range(16):
        m = np.exp(-2j * np.pi * (np.outer(n, n) / 128 + a * n[None, :] / S))
        ms.append(np.block([[m.real, m.imag]]))
    c = lambda v: np.asarray(v, np.float32).astype(bf16)
    return c(fd), c(gd), c(np.stack(ms))


def _fft(v, sg):
    n = len(v)
    if n == 1:
        return v
    e, o = _fft(v[0::2], sg), _fft(v[1::2], sg)
    out = [None] * n
    for k in range(n // 2):
        (er, ei), (a, b) = e[k], o[k]
        if k == 0:
            tr, ti = a, b
        elif 4 * k == n:
            if sg < 0:
                out[k], out[k + n // 2] = (er + b, ei - a), (er - b, ei + a)
            else:
                out[k], out[k + n // 2] = (er - b, ei + a), (er + b, ei - a)
            continue
        else:
            c, s = np.cos(2 * np.pi * k / n), sg * np.sin(2 * np.pi * k / n)
            if 8 * k == n:
                tr, ti = ((a - b) * c, (a + b) * c) if s > 0 else ((a + b) * c, (b - a) * c)
            elif 8 * k == 3 * n:
                tr, ti = ((a + b) * c, (b - a) * c) if s > 0 else ((a - b) * c, (a + b) * c)
            else:
                tr, ti = a * c - b * s, a * s + b * c
        out[k], out[k + n // 2] = (er + tr, ei + ti), (er - tr, ei - ti)
    return out


def _nt(a, b):
    return jax.lax.dot_general(a, b, (((1,), (1,)), ((), ())), preferred_element_type=f32)


def _nn(a, b):
    return jnp.dot(a, b, preferred_element_type=f32)


def _body(x_h, wr_h, wi_h, w1_h, w3_h, w2_h, fd_h, gd_h, m_h, o_h,
          x_v, wr_v, wi_v, w1, w3, w2, fd, gd, m, m2, xn_v, p_v, wf, z, acc, sem, osem):
    NT = S // TM
    xc = [pltpu.make_async_copy(x_h.at[pl.ds(i * TM, TM)], x_v.at[pl.ds(i * TM, TM)], sem.at[i])
          for i in range(NT)]
    rest = [pltpu.make_async_copy(a, b, sem.at[NT + i]) for i, (a, b) in enumerate(
        [(fd_h, fd), (m_h, m), (wr_h, wr_v), (wi_h, wi_v), (w1_h, w1), (w3_h, w3), (w2_h, w2), (gd_h, gd)])]
    for c in xc + rest[:2]:
        c.start()

    @pl.loop(0, NT,unroll=2)
    def _(i):
        r0 = pl.multiple_of(i * TM, TM)
        pltpu.make_async_copy(x_h.at[pl.ds(r0, TM)], x_v.at[pl.ds(r0, TM)], sem.at[i]).wait()
        x = x_v[pl.ds(r0, TM), :].astype(f32)
        c = x - jnp.mean(x, -1, keepdims=True)
        xn = c * jax.lax.rsqrt(jnp.mean(c * c, -1, keepdims=True) + 1e-5)
        xn_v[pl.ds(r0, TM), :] = xn.astype(bf16)
        x0, x1, x2, x3 = [xn[:, 128 * k:128 * k + 128] for k in range(4)]
        e, o = x0 + x2, x1 + x3
        for k, v in enumerate([e + o, e - o, x0 - x2, x1 - x3]):
            for b in range(16):
                p_v[k, pl.ds(i * 272 + 17 * b, 16), :] = v[16 * b:16 * b + 16]

    for c in rest[4:]:
        c.start()
    rest[0].wait(); rest[1].wait()
    sub0 = jax.lax.broadcasted_iota(jnp.int32, (8, 128), 0) == 0
    zero = jnp.zeros((8, 128), f32)

    def dd(a):
        p, q, r, t = [p_v[k, pl.ds(a, 128, stride=17), :].astype(bf16) for k in range(4)]
        y0 = _nt(fd[0:128, 0:128], p)
        y2 = _nt(fd[0:128, 128:256], q)
        y1 = _nt(fd[128:384, :], jnp.concatenate([r, t], 1))
        h = y0[64:72]
        re = jnp.concatenate([y0[:64], y2[:64], y1[:128], jnp.where(sub0, h, 0.0)], 0)
        im = jnp.concatenate([jnp.where(sub0, 0.0, h), y0[72:], y2[64:], y1[128:], zero], 0)
        return jnp.concatenate([re, im], 1).astype(bf16)

    cur = dd(0)
    for a in range(16):
        nxt = dd(a + 1) if a < 15 else None
        m2[a, 0:128, :] = m[a]
        m2[a, 128:256, 0:128] = -m[a, :, 128:256]
        m2[a, 128:256, 128:256] = m[a, :, 0:128]
        z[a] = _nn(cur, m2[a])
        cur = nxt

    def mid(g, wsl):
        v = _fft([(z[a, pl.ds(g, 8), 0:128], z[a, pl.ds(g, 8), 128:256]) for a in range(16)], -1)
        u = []
        for k, (a, b) in enumerate(v):
            c, d = wf[0, k, wsl, :], wf[1, k, wsl, :]
            u.append((a * c - b * d, a * d + b * c))
        for a, (re, im) in enumerate(_fft(u, 1)):
            z[a, pl.ds(g, 8), 0:128] = re
            z[a, pl.ds(g, 8), 128:256] = im

    for c in rest[4:]:
        c.wait()
    rest[2].start(); rest[3].start()

    def ffn(r0):
        xn = xn_v[pl.ds(r0, TM), :]
        g, u = _nt(xn, w1[...]), _nt(xn, w3[...])
        h = (g * u * pl.reciprocal(1.0 + jnp.exp(-g), approx=False)).astype(bf16)
        return x_v[pl.ds(r0, TM), :].astype(f32) + _nn(h, w2[...])

    acc[6 * TM:7 * TM, :] = ffn(6 * TM)
    rest[2].wait(); rest[3].wait()
    for k, w in enumerate((wr_v, wi_v)):
        @pl.loop(0, 16, unroll=4)
        def _(c):
            c0 = pl.multiple_of(c * 128, 128)
            wf[k, c, 0:256, :] = w[0:256, pl.ds(c0, 128)].astype(f32)
            wf[k, c, 256:264, :] = jnp.where(
                sub0, jnp.broadcast_to(w[256:257, pl.ds(c0, 128)].astype(f32), (8, 128)), 0.0)

    mid(256, pl.ds(256, 8))
    NA = 4
    @pl.loop(0, NA,unroll=2)
    def _(i):
        r0 = pl.multiple_of(i * TM, TM)
        off = ((i & 1) << 1) | (i >> 1)
        acc[pl.ds(r0, TM), :] = ffn(r0)
        for j in range(8):
            mid(pl.multiple_of(i * 64 + j * 8, 8), pl.ds(off + 32 * j, 8, stride=4))

    @pl.loop(NA, NA + 2)
    def _(i):
        r0 = pl.multiple_of(i * TM, TM)
        for j in range(8):
            a = (i - NA) * 8 + j
            y = _nt(z[a].astype(bf16), m2[a]) * (1.0 / S)
            re, im = y[:, :128], y[:, 128:]
            im0 = jnp.where(sub0, re[256:264], im[0:8])
            parts = [jnp.concatenate([re[0:64], im0, im[8:64]], 0),
                     jnp.concatenate([re[64:128], im[64:128]], 0), re[128:256], im[128:256]]
            for k, v in enumerate(parts):
                p_v[k, pl.ds(a, 128, stride=17), :] = v.T
        acc[pl.ds(r0, TM), :] = ffn(r0)

    def fin(t, base):
        r0 = t * TM if isinstance(t, int) else pl.multiple_of(t * TM, TM)
        y = [jnp.concatenate([p_v[k, pl.ds(t * 272 + 17 * b, 16), :] for b in range(16)], 0).astype(bf16)
             for k in range(4)]
        p = _nn(y[0], gd[0:128, 0:128])
        q = _nn(y[1], gd[0:128, 128:256])
        rt = _nn(jnp.concatenate(y[2:], 1), gd[128:384, :])
        r, s = rt[:, :128], rt[:, 128:]
        e, o = p + q, p - q
        res = base + jnp.concatenate([e + r, o + s, e - r, o - s], 1)
        x_v[pl.ds(r0, TM), :] = res.astype(bf16)

    oc = lambda t: pltpu.make_async_copy(x_v.at[pl.ds(t * TM, TM)], o_h.at[pl.ds(t * TM, TM)], osem.at[t])
    for t in range(7):
        fin(t, acc[t * TM:(t + 1) * TM, :])
    for t in range(7):
        oc(t).start()
    fin(7, ffn(7 * TM))
    oc(7).start()
    for t in range(8):
        oc(t).wait()


@jax.jit
def pallas_parallel_sum__spectral_gfnet__glu_gated_swiglu__prompt_kernel(
        A_x, A_w_r, A_w_i, B_x, B_w1, B_w3, B_w2):
    fd, gd, m = _consts()
    V = pltpu.VMEM
    out = pl.pallas_call(
        _body,
        in_specs=[pl.BlockSpec(memory_space=pl.ANY)] * 9,
        out_specs=pl.BlockSpec(memory_space=pl.ANY),
        out_shape=jax.ShapeDtypeStruct((S, D), bf16),
        scratch_shapes=[
            V((S, D), bf16), V((257, S), bf16), V((257, S), bf16),
            V((F, D), bf16), V((F, D), bf16), V((F, D), bf16),
            V(fd.shape, bf16), V(gd.shape, bf16), V(m.shape, bf16), V((16, 256, 256), bf16),
            V((S, D), bf16), V((4, 17 * 128, 128), f32), V((2, 16, R, 128), f32),
            V((16, R, 256), f32), V((S, D), f32),
            pltpu.SemaphoreType.DMA((16,)), pltpu.SemaphoreType.DMA((8,))],
        compiler_params=pltpu.CompilerParams(vmem_limit_bytes=100 << 20),
    )(A_x.reshape(S, D), A_w_r.T, A_w_i.T, B_w1.T, B_w3.T, B_w2, fd, gd, m)
    return out.reshape(1, S, D)
```
